```python
import os as _os
_os.environ.setdefault("JAX_PLATFORMS", "cpu")
import jax
import jax.numpy as jnp

def _softmax(x, axis=-1):
    return jax.nn.softmax(x, axis=axis)
def _gelu(x):
    return jax.nn.gelu(x, approximate=True)
def _silu(x):
    return jax.nn.silu(x)
def _sigmoid(x):
    return jax.nn.sigmoid(x)
def _layernorm(x, axis=-1, eps=1e-5):
    m = jnp.mean(x, axis=axis, keepdims=True)
    v = jnp.var(x, axis=axis, keepdims=True)
    return (x - m) / jnp.sqrt(v + eps)
def _scatter_add(tgt, idx, src, axis=0):
    return tgt.at[idx].add(src)
def _segment_sum(src, seg, n):
    return jax.ops.segment_sum(src, seg, n)
class _Rng:
    def __init__(self, key):
        self._k = key
    def _next(self):
        self._k, sub = jax.random.split(self._k)
        return sub
    def normal(self, shape):
        return jax.random.normal(self._next(), shape, dtype=jnp.bfloat16)
    def randint(self, lo, hi, shape):
        return jax.random.randint(self._next(), shape, lo, hi, dtype=jnp.int32)
    def uniform(self, shape, lo=0.0, hi=1.0):
        return jax.random.uniform(self._next(), shape, jnp.bfloat16, lo, hi)
    def permutation(self, n):
        return jax.random.permutation(self._next(), n)


kernel_name = 'standalone__gqa_block_cached__near_ridge'

def setup_inputs():
    _rng = _Rng(jax.random.key(int.from_bytes(__import__("os").urandom(4), "little")))
    _w = (lambda a: (lambda t: t.astype(jnp.bfloat16) if jnp.issubdtype(t.dtype, jnp.floating) else t)(jnp.asarray(a)))
    B, Sq, D = 16, 128, 576
    Hq, Hkv, Sk, Dh = 32, 16, 1024, 128
    assert Hq % Hkv == 0, (Hq, Hkv)
    return {
        "x": _w((lambda *s: _rng.normal(s) * 0.8)(B, Sq, D)),
        "k_cache": _w((lambda *s: _rng.normal(s) * 0.8)(B, Hkv, Sk, Dh)),
        "v_cache": _w((lambda *s: _rng.normal(s) * 0.05)(B, Hkv, Sk, Dh)),
        "wq": _w((lambda *s: _rng.normal(s) * 0.8)(D, Hq * Dh) * (D ** -0.5)),
        "wo": _w((lambda *s: _rng.normal(s) * 0.05)(Hq * Dh, D) * ((Hq * Dh) ** -0.5)),
    }

def reference(x, k_cache, v_cache, wq, wo):
    B, Sq, D = x.shape
    Hq, Dh = 32, 128
    Hkv = k_cache.shape[1]
    rep = Hq // Hkv
    q = (lambda x, *d: x.transpose(*d))((x @ wq).reshape(B, Sq, Hq, Dh), 0, 2, 1, 3)
    k = jnp.repeat(k_cache, rep, axis=1)
    v = jnp.repeat(v_cache, rep, axis=1)
    scores = jnp.einsum("bhqd,bhkd->bhqk", q, k) * (Dh ** -0.5)
    p = _softmax(scores, axis=-1)
    o = jnp.einsum("bhqk,bhkd->bhqd", p, v)
    return (lambda x, *d: x.transpose(*d))(o, 0, 2, 1, 3).reshape(B, Sq, Hq * Dh) @ wo
```

```python
import functools

import jax
import jax.numpy as jnp
import jax.experimental.pallas as pl
import jax.experimental.pallas.tpu as pltpu


def _gqa_kernel(x_ref, k_ref, v_ref, wq_ref, wo_ref, o_ref, acc_ref, *, hb, rep, dh, sq, scale):
    h = pl.program_id(1)
    x = x_ref[0]
    q_all = jnp.dot(x, wq_ref[...], preferred_element_type=jnp.float32)
    q_all = (q_all * scale).astype(jnp.bfloat16)
    outs = []
    for j in range(hb):
        q = jnp.concatenate(
            [q_all[:, (j * rep + r) * dh:(j * rep + r + 1) * dh] for r in range(rep)], axis=0)
        k = k_ref[0, j]
        v = v_ref[0, j]
        s = jax.lax.dot_general(q, k, (((1,), (1,)), ((), ())),
                                preferred_element_type=jnp.float32)
        m = jnp.max(s, axis=-1, keepdims=True)
        p = jnp.exp(s - m)
        l = jnp.sum(p, axis=-1, keepdims=True)
        o = jnp.dot(p.astype(jnp.bfloat16), v, preferred_element_type=jnp.float32)
        o = (o / l).astype(jnp.bfloat16)
        for r in range(rep):
            outs.append(o[r * sq:(r + 1) * sq])
    o_all = jnp.concatenate(outs, axis=1)
    part = jnp.dot(o_all, wo_ref[...], preferred_element_type=jnp.float32)

    @pl.when(h == 0)
    def _():
        acc_ref[...] = part

    @pl.when(h != 0)
    def _():
        acc_ref[...] += part

    @pl.when(h == pl.num_programs(1) - 1)
    def _():
        o_ref[0] = acc_ref[...].astype(o_ref.dtype)


@jax.jit
def pallas_standalone__gqa_block_cached__near_ridge_kernel(
    x: jax.Array,
    k_cache: jax.Array,
    v_cache: jax.Array,
    wq: jax.Array,
    wo: jax.Array,
):
    B, Sq, D = x.shape
    _, Hkv, Sk, Dh = k_cache.shape
    Hq = wq.shape[1] // Dh
    rep = Hq // Hkv
    hb = 4
    nh = Hkv // hb
    cols = hb * rep * Dh
    kernel = functools.partial(_gqa_kernel, hb=hb, rep=rep, dh=Dh, sq=Sq, scale=float(Dh) ** -0.5)
    return pl.pallas_call(
        kernel,
        grid=(B, nh),
        in_specs=[
            pl.BlockSpec((1, Sq, D), lambda b, h: (b, 0, 0)),
            pl.BlockSpec((1, hb, Sk, Dh), lambda b, h: (b, h, 0, 0)),
            pl.BlockSpec((1, hb, Sk, Dh), lambda b, h: (b, h, 0, 0)),
            pl.BlockSpec((D, cols), lambda b, h: (0, h)),
            pl.BlockSpec((cols, D), lambda b, h: (h, 0)),
        ],
        out_specs=pl.BlockSpec((1, Sq, D), lambda b, h: (b, 0, 0)),
        out_shape=jax.ShapeDtypeStruct((B, Sq, D), x.dtype),
        scratch_shapes=[pltpu.VMEM((Sq, D), jnp.float32)],
        compiler_params=pltpu.CompilerParams(
            dimension_semantics=("arbitrary", "arbitrary"),
            vmem_limit_bytes=100 * 1024 * 1024,
        ),
    )(x, k_cache, v_cache, wq, wo)
```

```python
import functools

import jax
import jax.numpy as jnp
import jax.experimental.pallas as pl
import jax.experimental.pallas.tpu as pltpu


def _gqa_kernel(xt_ref, k_ref, v_ref, wq_ref, wot_ref, o_ref, acc_ref, *, hb, rep, dh, sq, scale):
    h = pl.program_id(1)
    cols = hb * rep * dh
    c0 = pl.multiple_of(h * cols, cols)
    x = xt_ref[0].T
    q_all = jnp.dot(x, wq_ref[:, pl.ds(c0, cols)], preferred_element_type=jnp.float32)
    q_all = (q_all * scale).astype(jnp.bfloat16)
    outs = []
    for j in range(hb):
        q = jnp.concatenate(
            [q_all[:, (j * rep + r) * dh:(j * rep + r + 1) * dh] for r in range(rep)], axis=0)
        k = k_ref[0, j]
        v = v_ref[0, j]
        s = jax.lax.dot_general(q, k, (((1,), (1,)), ((), ())),
                                preferred_element_type=jnp.float32)
        m = jnp.max(s, axis=-1, keepdims=True)
        p = jnp.exp(s - m)
        l = jnp.sum(p, axis=-1, keepdims=True)
        o = jnp.dot(p.astype(jnp.bfloat16), v, preferred_element_type=jnp.float32)
        o = (o / l).astype(jnp.bfloat16)
        for r in range(rep):
            outs.append(o[r * sq:(r + 1) * sq])
    o_all = jnp.concatenate(outs, axis=1)
    part = jax.lax.dot_general(wot_ref[:, pl.ds(c0, cols)], o_all, (((1,), (1,)), ((), ())),
                               preferred_element_type=jnp.float32)

    @pl.when(h == 0)
    def _():
        acc_ref[...] = part

    @pl.when(h != 0)
    def _():
        acc_ref[...] += part

    @pl.when(h == pl.num_programs(1) - 1)
    def _():
        o_ref[0] = acc_ref[...].astype(o_ref.dtype)


@jax.jit
def pallas_standalone__gqa_block_cached__near_ridge_kernel(
    x: jax.Array,
    k_cache: jax.Array,
    v_cache: jax.Array,
    wq: jax.Array,
    wo: jax.Array,
):
    B, Sq, D = x.shape
    _, Hkv, Sk, Dh = k_cache.shape
    Hq = wq.shape[1] // Dh
    rep = Hq // Hkv
    hb = 8
    nh = Hkv // hb
    kernel = functools.partial(_gqa_kernel, hb=hb, rep=rep, dh=Dh, sq=Sq, scale=float(Dh) ** -0.5)
    out_t = pl.pallas_call(
        kernel,
        grid=(B, nh),
        in_specs=[
            pl.BlockSpec((1, D, Sq), lambda b, h: (b, 0, 0)),
            pl.BlockSpec((1, hb, Sk, Dh), lambda b, h: (b, h, 0, 0)),
            pl.BlockSpec((1, hb, Sk, Dh), lambda b, h: (b, h, 0, 0)),
            pl.BlockSpec((D, Hq * Dh), lambda b, h: (0, 0)),
            pl.BlockSpec((D, Hq * Dh), lambda b, h: (0, 0)),
        ],
        out_specs=pl.BlockSpec((1, D, Sq), lambda b, h: (b, 0, 0)),
        out_shape=jax.ShapeDtypeStruct((B, D, Sq), x.dtype),
        scratch_shapes=[pltpu.VMEM((D, Sq), jnp.float32)],
        compiler_params=pltpu.CompilerParams(
            dimension_semantics=("arbitrary", "arbitrary"),
            vmem_limit_bytes=100 * 1024 * 1024,
        ),
    )(x.transpose(0, 2, 1), k_cache, v_cache, wq, wo.T)
    return out_t.transpose(0, 2, 1)
```
